```python
import jax
import jax.numpy as jnp

def _softmax(x, axis=-1):
    return jax.nn.softmax(x, axis=axis)
def _gelu(x):
    return jax.nn.gelu(x, approximate=True)
def _silu(x):
    return jax.nn.silu(x)
def _sigmoid(x):
    return jax.nn.sigmoid(x)
def _layernorm(x, axis=-1, eps=1e-5):
    m = jnp.mean(x, axis=axis, keepdims=True)
    v = jnp.var(x, axis=axis, keepdims=True)
    return (x - m) / jnp.sqrt(v + eps)
def _scatter_add(tgt, idx, src, axis=0):
    return tgt.at[idx].add(src)
def _segment_sum(src, seg, n):
    return jax.ops.segment_sum(src, seg, n)
class _Rng:
    def __init__(self, key):
        self._k = key
    def _next(self):
        self._k, sub = jax.random.split(self._k)
        return sub
    def normal(self, shape):
        return jax.random.normal(self._next(), shape, dtype=jnp.bfloat16)
    def randint(self, lo, hi, shape):
        return jax.random.randint(self._next(), shape, lo, hi, dtype=jnp.int32)
    def uniform(self, shape, lo=0.0, hi=1.0):
        return jax.random.uniform(self._next(), shape, jnp.bfloat16, lo, hi)
    def permutation(self, n):
        return jax.random.permutation(self._next(), n)


kernel_name = 'standalone__qk_norm__prompt'

def setup_inputs():
    _rng = _Rng(jax.random.key(int.from_bytes(__import__("os").urandom(4), "little")))
    _w = (lambda a: (lambda t: t.astype(jnp.bfloat16) if jnp.issubdtype(t.dtype, jnp.floating) else t)(jnp.asarray(a)))
    B, H, S, D = 2, 32, 2048, 1024
    Dh = D // H
    return {
        "q": _w((lambda *s: _rng.normal(s) * 0.05)(B, H, S, Dh)),
        "k": _w((lambda *s: _rng.normal(s) * 0.05)(B, H, S, Dh)),
        "v": _w((lambda *s: _rng.normal(s) * 0.05)(B, H, S, Dh)),
        "t": _w(jnp.abs((lambda *s: _rng.normal(s) * 0.05)(H)) + 1.0),
    }

def reference(q, k, v, t):
    eps = 1e-6
    qn = q / (jnp.sqrt((q * q).sum(axis=-1, keepdims=True)) + eps)
    kn = k / (jnp.sqrt((k * k).sum(axis=-1, keepdims=True)) + eps)
    logits = jnp.einsum('bhqd,bhkd->bhqk', qn, kn) * t[None, :, None, None]
    attn = _softmax(logits, axis=-1)
    return jnp.einsum('bhqk,bhkd->bhqd', attn, v)
```

```python
import jax
import jax.numpy as jnp
import jax.experimental.pallas as pl
import jax.experimental.pallas.tpu as pltpu

_LOG2E = 1.4426950408889634
_EPS = 1e-6
_T_SAFE = 16.0
_BQ = 1024
_BQS = 512
_HPS = 4


def _unit(x):
    return x / (jnp.sqrt(jnp.sum(x * x, axis=0, keepdims=True)) + _EPS)


def _kernel(t_ref, q_ref, k_ref, v_ref, o_ref, kn_ref):
    S = k_ref.shape[-1]
    h0 = pl.program_id(1) * _HPS
    tmax = jnp.abs(t_ref[h0])
    for hh in range(1, _HPS):
        tmax = jnp.maximum(tmax, jnp.abs(t_ref[h0 + hh]))
    safe = tmax <= _T_SAFE

    @pl.when(safe)
    def _fast():
        for hh in range(_HPS):
            kn_ref[hh] = _unit(k_ref[hh].astype(jnp.float32)).T.astype(jnp.bfloat16)
            tval = t_ref[h0 + hh] * _LOG2E
            for i in range(S // _BQ):
                rs = pl.ds(i * _BQ, _BQ)
                qn = (_unit(q_ref[hh, :, rs].astype(jnp.float32)) * tval).astype(jnp.bfloat16)
                p = jnp.exp2(jnp.dot(kn_ref[hh], qn, preferred_element_type=jnp.float32))
                l = jnp.sum(p, axis=0, keepdims=True)
                acc = jnp.dot(v_ref[hh], p.astype(jnp.bfloat16), preferred_element_type=jnp.float32)
                o_ref[hh, :, rs] = (acc / l).astype(o_ref.dtype)

    @pl.when(jnp.logical_not(safe))
    def _slow():
        def head(hh, carry):
            kn_ref[0] = _unit(k_ref[hh].astype(jnp.float32)).T.astype(jnp.bfloat16)
            tval = t_ref[h0 + hh] * _LOG2E

            def rtile(i, c):
                rs = pl.ds(pl.multiple_of(i * _BQS, _BQS), _BQS)
                qn = _unit(q_ref[hh, :, rs].astype(jnp.float32)).astype(jnp.bfloat16)
                s = jnp.dot(kn_ref[0], qn, preferred_element_type=jnp.float32) * tval
                p = jnp.exp2(s - jnp.max(s, axis=0, keepdims=True))
                l = jnp.sum(p, axis=0, keepdims=True)
                acc = jnp.dot(v_ref[hh], p.astype(jnp.bfloat16), preferred_element_type=jnp.float32)
                o_ref[hh, :, rs] = (acc / l).astype(o_ref.dtype)
                return c

            jax.lax.fori_loop(0, S // _BQS, rtile, 0)
            return carry

        jax.lax.fori_loop(0, _HPS, head, 0)


@jax.jit
def pallas_standalone__qk_norm__prompt_kernel(
    q: jax.Array,
    k: jax.Array,
    v: jax.Array,
    t: jax.Array,
):
    B, H, S, Dh = q.shape
    qt = jnp.swapaxes(q, 2, 3)
    kt = jnp.swapaxes(k, 2, 3)
    vt = jnp.swapaxes(v, 2, 3)
    spec = pl.BlockSpec((None, _HPS, Dh, S), lambda b, h: (b, h, 0, 0))
    out = pl.pallas_call(
        _kernel,
        grid=(B, H // _HPS),
        in_specs=[pl.BlockSpec(memory_space=pltpu.SMEM), spec, spec, spec],
        out_specs=spec,
        out_shape=jax.ShapeDtypeStruct((B, H, Dh, S), q.dtype),
        scratch_shapes=[pltpu.VMEM((_HPS, S, Dh), jnp.bfloat16)],
        compiler_params=pltpu.CompilerParams(
            dimension_semantics=("parallel", "parallel"),
            vmem_limit_bytes=64 * 1024 * 1024,
        ),
    )(t.astype(jnp.float32), qt, kt, vt)
    return jnp.swapaxes(out, 2, 3)
```

```python
import jax
import jax.numpy as jnp
import jax.experimental.pallas as pl
import jax.experimental.pallas.tpu as pltpu

_LOG2E = 1.4426950408889634
_EPS = 1e-6
_T_SAFE = 16.0
_MAGIC = 12582912.0

_HPS = 4
_BQ = 1024
_CK = 128
_DT = 128
_BQS = 512

_SCHED = dict(qs=[0], ks=[2], qd=[4, 5, 6, 7, 8, 9, 10, 11],
              kd=[6, 7, 8, 9, 10, 11, 12, 13])


def _unit(x):
    return x / (jnp.sqrt(jnp.sum(x * x, axis=0, keepdims=True)) + _EPS)


def _inv_norm(x):
    y = jax.lax.rsqrt(jnp.maximum(jnp.sum(x * x, axis=0, keepdims=True), 1e-36))
    return y * pltpu.reciprocal(1.0 + _EPS * y, approx=True)


def _k_scale(kf):
    return _inv_norm(kf) * 4064.0


def _k_digits(kf, inv):
    t = pltpu.bitcast(kf * inv + (_MAGIC + 8.0), jnp.int32)
    planes = [t >> 5, (t + 16) >> 5, (t & 15) - 8, (t + 120) >> 8]
    return jnp.concatenate(planes, axis=0).T.astype(jnp.int8)


def _q_scale(qf):
    amax = jnp.maximum(jnp.max(jnp.abs(qf), axis=0, keepdims=True), 1e-30)
    return pltpu.reciprocal(amax, approx=True) * 2032.0, amax * _inv_norm(qf)


def _q_digits(qf, r):
    t = pltpu.bitcast(qf * r + (_MAGIC + 4.0), jnp.int32)
    planes = [t >> 4, (t + 8) >> 4, (t + 124) >> 8, (t & 7) - 4]
    return jnp.concatenate(planes, axis=0).astype(jnp.int8)


def _zero_from(*vals):
    acc = None
    for v in vals:
        w = pltpu.bitcast(v, jnp.int32)
        if w.shape[0] == 1:
            w = jnp.broadcast_to(w, (8, w.shape[1]))
        for i in range(0, w.shape[0], 8):
            for j in range(0, w.shape[1], 128):
                x = w[i:i + 8, j:j + 128]
                acc = x if acc is None else acc | x
    zero = jnp.minimum(jax.lax.shift_right_logical(acc, 1), 0)
    return pltpu.bitcast(zero, jnp.float32)


def _kernel(t_ref, q_ref, k_ref, v_ref, qx_ref, kx_ref, o_ref,
            kd_ref, kn_ref, qd_ref, qm_ref, flag_ref):
    S = k_ref.shape[-1]
    H = t_ref.shape[0]
    step = pl.program_id(0)
    h0 = (step * _HPS) % H

    @pl.when(step == 0)
    def _prologue():
        tmax = jnp.abs(t_ref[0])
        for h in range(1, H):
            tmax = jnp.maximum(tmax, jnp.abs(t_ref[h]))
        flag_ref[0] = (tmax <= _T_SAFE).astype(jnp.int32)
        kf = k_ref[0].astype(jnp.float32)
        kd_ref[...] = _k_digits(kf, _k_scale(kf))
        qf = q_ref[0, :, pl.ds(0, _BQ)].astype(jnp.float32)
        r, m = _q_scale(qf)
        qd_ref[...] = _q_digits(qf, r)
        qm_ref[...] = m

    safe = flag_ref[0] == 1

    @pl.when(safe)
    def _bounded_logits():
        n_c, n_r, n_d = S // _CK, S // _BQ, _BQ // _DT
        items = [(hh, i, c) for hh in range(_HPS) for i in range(n_r) for c in range(n_c)]
        P, L, ACC, SC, QD, QS, KS, KD = {}, {}, {}, {}, {}, {}, {}, {}
        at = {}
        for kind, pos in _SCHED.items():
            for j, c in enumerate(pos):
                at.setdefault(c, []).append((kind, j))

        def k_src(hh):
            return k_ref.at[hh + 1] if hh + 1 < _HPS else kx_ref.at[0]

        def q_src(hh, i):
            if i + 1 < n_r:
                return q_ref.at[hh], (i + 1) * _BQ
            return (q_ref.at[hh + 1] if hh + 1 < _HPS else qx_ref.at[0]), 0

        def prepare(n):
            hh, i, c = items[n]
            u = hh * n_r + i
            q_nxt, base = q_src(hh, i)
            outs = []
            for kind, j in at.get(c, []):
                cols = slice(j * _DT, (j + 1) * _DT)
                if kind == "ks":
                    KS[u] = _k_scale(k_src(hh)[:, pl.ds(i * _BQ, _BQ)].astype(jnp.float32))
                    outs.append(KS[u])
                elif kind == "qs":
                    QS[u] = _q_scale(q_nxt[:, pl.ds(base, _BQ)].astype(jnp.float32))
                    outs += list(QS[u])
                elif kind == "kd":
                    kf = k_src(hh)[:, pl.ds(i * _BQ + j * _DT, _DT)].astype(jnp.float32)
                    KD[hh + 1, i * n_d + j] = _k_digits(kf, KS[u][:, cols])
                    outs.append(KD[hh + 1, i * n_d + j])
                else:
                    qf = q_nxt[:, pl.ds(base + j * _DT, _DT)].astype(jnp.float32)
                    QD[u + 1, j] = _q_digits(qf, QS[u][0][:, cols])
                    outs.append(QD[u + 1, j])
            return outs

        def scores(n):
            hh, i, c = items[n]
            u = hh * n_r + i
            if c == 0:
                if u == 0:
                    QD[u], m = qd_ref[...], qm_ref[...]
                else:
                    QD[u] = jnp.concatenate([QD[u, j] for j in range(n_d)], axis=1)
                    m = QS[u - 1][1]
                SC[u] = m * (t_ref[h0 + hh] * (_LOG2E / 32258.0))
            kd = kd_ref[pl.ds(c * _CK, _CK), :] if hh == 0 else KD[hh, c]
            s = jnp.dot(kd, QD[u], preferred_element_type=jnp.int32)
            p = jnp.exp2(s.astype(jnp.float32) * SC[u])
            P[n] = p.astype(jnp.bfloat16)
            ls = jnp.sum(p.reshape(_CK // 8, 8, _BQ), axis=0)
            L[hh, i] = ls if c == 0 else L[hh, i] + ls

        def values(n):
            hh, i, c = items[n]
            a = jnp.dot(v_ref[hh, :, pl.ds(c * _CK, _CK)], P.pop(n),
                        preferred_element_type=jnp.float32)
            outs = prepare(n)
            if outs:
                top = jnp.concatenate([a[:8, :128] + _zero_from(*outs), a[:8, 128:]], axis=1)
                a = jnp.concatenate([top, a[8:]], axis=0)
            ACC[hh, i] = a if c == 0 else ACC[hh, i] + a
            if c == n_c - 1:
                l = jnp.sum(L.pop((hh, i)), axis=0, keepdims=True)
                o_ref[hh, :, pl.ds(i * _BQ, _BQ)] = (ACC.pop((hh, i)) / l).astype(o_ref.dtype)

        for n in range(len(items) + 1):
            if n < len(items):
                scores(n)
            if n >= 1:
                values(n - 1)

        for j in range(S // _DT):
            kd_ref[pl.ds(j * _DT, _DT), :] = KD[_HPS, j]
        for j in range(n_d):
            qd_ref[:, pl.ds(j * _DT, _DT)] = QD[_HPS * n_r, j]
        qm_ref[...] = QS[_HPS * n_r - 1][1]

    @pl.when(jnp.logical_not(safe))
    def _true_max():
        def head(hh, carry):
            kn_ref[...] = _unit(k_ref[hh].astype(jnp.float32)).T.astype(jnp.bfloat16)
            tval = t_ref[h0 + hh] * _LOG2E

            def rtile(i, c):
                rs = pl.ds(pl.multiple_of(i * _BQS, _BQS), _BQS)
                qn = _unit(q_ref[hh, :, rs].astype(jnp.float32)).astype(jnp.bfloat16)
                s = jnp.dot(kn_ref[...], qn, preferred_element_type=jnp.float32) * tval
                p = jnp.exp2(s - jnp.max(s, axis=0, keepdims=True))
                l = jnp.sum(p, axis=0, keepdims=True)
                acc = jnp.dot(v_ref[hh], p.astype(jnp.bfloat16), preferred_element_type=jnp.float32)
                o_ref[hh, :, rs] = (acc / l).astype(o_ref.dtype)
                return c

            jax.lax.fori_loop(0, S // _BQS, rtile, 0)
            return carry

        jax.lax.fori_loop(0, _HPS, head, 0)


@jax.jit
def pallas_standalone__qk_norm__prompt_kernel(
    q: jax.Array,
    k: jax.Array,
    v: jax.Array,
    t: jax.Array,
):
    B, H, S, Dh = q.shape
    BH = B * H
    assert Dh == 32 and S % _BQ == 0 and H % _HPS == 0 and _CK == _DT
    qt = jnp.swapaxes(q, 2, 3).reshape(BH, Dh, S)
    kt = jnp.swapaxes(k, 2, 3).reshape(BH, Dh, S)
    vt = jnp.swapaxes(v, 2, 3).reshape(BH, Dh, S)
    spec = pl.BlockSpec((_HPS, Dh, S), lambda g: (g, 0, 0))
    nxt = lambda g: (jnp.minimum((g + 1) * _HPS, BH - 1), 0, 0)
    out = pl.pallas_call(
        _kernel,
        grid=(BH // _HPS,),
        in_specs=[pl.BlockSpec(memory_space=pltpu.SMEM), spec, spec, spec,
                  pl.BlockSpec((1, Dh, _BQ), nxt), pl.BlockSpec((1, Dh, S), nxt)],
        out_specs=spec,
        out_shape=jax.ShapeDtypeStruct((BH, Dh, S), q.dtype),
        scratch_shapes=[
            pltpu.VMEM((S, 4 * Dh), jnp.int8),
            pltpu.VMEM((S, Dh), jnp.bfloat16),
            pltpu.VMEM((4 * Dh, _BQ), jnp.int8),
            pltpu.VMEM((1, _BQ), jnp.float32),
            pltpu.SMEM((1,), jnp.int32),
        ],
        compiler_params=pltpu.CompilerParams(
            dimension_semantics=("arbitrary",),
            vmem_limit_bytes=100 * 1024 * 1024,
        ),
    )(t.astype(jnp.float32), qt, kt, vt, qt, kt)
    return jnp.swapaxes(out.reshape(B, H, Dh, S), 2, 3)
```

```python
import jax
import jax.numpy as jnp
import jax.experimental.pallas as pl
import jax.experimental.pallas.tpu as pltpu

_LOG2E = 1.4426950408889634
_EPS = 1e-6
_T_SAFE = 16.0
_MAGIC = 12582912.0

_HPS = 4
_BQ = 1024
_CK = 128
_DT = 128
_BQS = 512

_SCHED = dict(qs=[0], ks=[2], qd=[4, 5, 6, 7, 8, 9, 10, 11],
              kd=[6, 7, 8, 9, 10, 11, 12, 13])


def _unit(x):
    return x / (jnp.sqrt(jnp.sum(x * x, axis=0, keepdims=True)) + _EPS)


def _compact(x):
    rows = jax.lax.broadcasted_iota(jnp.int32, (8, 128), 0)
    c = jnp.broadcast_to(x[:, 0:128], (8, 128))
    for s in range(1, x.shape[1] // 128):
        c = jnp.where(rows == s, jnp.broadcast_to(x[:, s * 128:(s + 1) * 128], (8, 128)), c)
    return c


def _expand(c, n):
    return jnp.concatenate([c[s:s + 1, :] for s in range(n)], axis=1)


def _inv_norm(ss):
    y = jax.lax.rsqrt(jnp.maximum(ss, 1e-36))
    return y * pltpu.reciprocal(1.0 + _EPS * y, approx=True)


def _k_scale(kf):
    ss = _compact(jnp.sum(kf * kf, axis=0, keepdims=True))
    return _expand(_inv_norm(ss) * 4064.0, kf.shape[1] // 128)


def _k_digits(kf, inv):
    t = pltpu.bitcast(kf * inv + (_MAGIC + 8.0), jnp.int32)
    planes = [t >> 5, (t + 16) >> 5, (t & 15) - 8, (t + 120) >> 8]
    return jnp.concatenate(planes, axis=0).T.astype(jnp.int8)


def _q_scale(qf):
    n = qf.shape[1] // 128
    sq = qf * qf
    inv = _inv_norm(_compact(jnp.sum(sq, axis=0, keepdims=True)))
    m2 = jnp.clip(_compact(jnp.max(sq, axis=0, keepdims=True)), 1e-36, 3.4028234e38)
    y = jax.lax.rsqrt(m2)
    return _expand(y * 2032.0, n), _expand(m2 * y * inv, n)


def _q_digits(qf, r):
    t = pltpu.bitcast(qf * r + (_MAGIC + 4.0), jnp.int32)
    planes = [t >> 4, (t + 8) >> 4, (t + 124) >> 8, (t & 7) - 4]
    return jnp.concatenate(planes, axis=0).astype(jnp.int8)


def _zero_from(*vals):
    acc = None
    for v in vals:
        w = pltpu.bitcast(v, jnp.int32)
        if w.shape[0] == 1:
            w = jnp.broadcast_to(w, (8, w.shape[1]))
        for i in range(0, w.shape[0], 8):
            for j in range(0, w.shape[1], 128):
                x = w[i:i + 8, j:j + 128]
                acc = x if acc is None else acc | x
    zero = jnp.minimum(jax.lax.shift_right_logical(acc, 1), 0)
    return pltpu.bitcast(zero, jnp.float32)


def _kernel(t_ref, q_ref, k_ref, v_ref, qx_ref, kx_ref, o_ref,
            kd_ref, kn_ref, qd_ref, qm_ref, flag_ref):
    S = k_ref.shape[-1]
    H = t_ref.shape[0]
    step = pl.program_id(0)
    h0 = (step * _HPS) % H

    @pl.when(step == 0)
    def _prologue():
        tmax = jnp.abs(t_ref[0])
        for h in range(1, H):
            tmax = jnp.maximum(tmax, jnp.abs(t_ref[h]))
        flag_ref[0] = (tmax <= _T_SAFE).astype(jnp.int32)
        for i in range(S // _BQ):
            kf = k_ref[0, :, pl.ds(i * _BQ, _BQ)].astype(jnp.float32)
            kd_ref[pl.ds(i * _BQ, _BQ), :] = _k_digits(kf, _k_scale(kf))
        qf = q_ref[0, :, pl.ds(0, _BQ)].astype(jnp.float32)
        r, m = _q_scale(qf)
        qd_ref[...] = _q_digits(qf, r)
        qm_ref[...] = m

    safe = flag_ref[0] == 1

    @pl.when(safe)
    def _bounded_logits():
        n_c, n_r, n_d = S // _CK, S // _BQ, _BQ // _DT
        items = [(hh, i, c) for hh in range(_HPS) for i in range(n_r) for c in range(n_c)]
        P, L, ACC, SC, QD, QS, KS, KD = {}, {}, {}, {}, {}, {}, {}, {}
        at = {}
        for kind, pos in _SCHED.items():
            for j, c in enumerate(pos):
                at.setdefault(c, []).append((kind, j))

        def k_src(hh):
            return k_ref.at[hh + 1] if hh + 1 < _HPS else kx_ref.at[0]

        def q_src(hh, i):
            if i + 1 < n_r:
                return q_ref.at[hh], (i + 1) * _BQ
            return (q_ref.at[hh + 1] if hh + 1 < _HPS else qx_ref.at[0]), 0

        def prepare(n):
            hh, i, c = items[n]
            u = hh * n_r + i
            q_nxt, base = q_src(hh, i)
            outs = []
            for kind, j in at.get(c, []):
                cols = slice(j * _DT, (j + 1) * _DT)
                if kind == "ks":
                    KS[u] = _k_scale(k_src(hh)[:, pl.ds(i * _BQ, _BQ)].astype(jnp.float32))
                    outs.append(KS[u])
                elif kind == "qs":
                    QS[u] = _q_scale(q_nxt[:, pl.ds(base, _BQ)].astype(jnp.float32))
                    outs += list(QS[u])
                elif kind == "kd":
                    kf = k_src(hh)[:, pl.ds(i * _BQ + j * _DT, _DT)].astype(jnp.float32)
                    KD[hh + 1, i * n_d + j] = _k_digits(kf, KS[u][:, cols])
                    outs.append(KD[hh + 1, i * n_d + j])
                else:
                    qf = q_nxt[:, pl.ds(base + j * _DT, _DT)].astype(jnp.float32)
                    QD[u + 1, j] = _q_digits(qf, QS[u][0][:, cols])
                    outs.append(QD[u + 1, j])
            return outs

        def scores(n):
            hh, i, c = items[n]
            u = hh * n_r + i
            if c == 0:
                if u == 0:
                    QD[u], m = qd_ref[...], qm_ref[...]
                else:
                    QD[u] = jnp.concatenate([QD[u, j] for j in range(n_d)], axis=1)
                    m = QS[u - 1][1]
                SC[u] = m * (t_ref[h0 + hh] * (_LOG2E / 32258.0))
            kd = kd_ref[pl.ds(c * _CK, _CK), :] if hh == 0 else KD[hh, c]
            s = jnp.dot(kd, QD[u], preferred_element_type=jnp.int32)
            p = jnp.exp2(s.astype(jnp.float32) * SC[u])
            P[n] = p.astype(jnp.bfloat16)
            ls = jnp.sum(p.reshape(_CK // 8, 8, _BQ), axis=0)
            L[hh, i] = ls if c == 0 else L[hh, i] + ls

        def values(n):
            hh, i, c = items[n]
            a = jnp.dot(v_ref[hh, :, pl.ds(c * _CK, _CK)], P.pop(n),
                        preferred_element_type=jnp.float32)
            outs = prepare(n)
            if outs:
                top = jnp.concatenate([a[:8, :-128], a[:8, -128:] + _zero_from(*outs)], axis=1)
                a = jnp.concatenate([top, a[8:]], axis=0)
            ACC[hh, i] = a if c == 0 else ACC[hh, i] + a
            if c == n_c - 1:
                l = jnp.sum(L.pop((hh, i)), axis=0, keepdims=True)
                o_ref[hh, :, pl.ds(i * _BQ, _BQ)] = (ACC.pop((hh, i)) / l).astype(o_ref.dtype)

        for n in range(len(items) + 1):
            if n < len(items):
                scores(n)
            if n >= 1:
                values(n - 1)

        for j in range(S // _DT):
            kd_ref[pl.ds(j * _DT, _DT), :] = KD[_HPS, j]
        for j in range(n_d):
            qd_ref[:, pl.ds(j * _DT, _DT)] = QD[_HPS * n_r, j]
        qm_ref[...] = QS[_HPS * n_r - 1][1]

    @pl.when(jnp.logical_not(safe))
    def _true_max():
        def head(hh, carry):
            kn_ref[...] = _unit(k_ref[hh].astype(jnp.float32)).T.astype(jnp.bfloat16)
            tval = t_ref[h0 + hh] * _LOG2E

            def rtile(i, c):
                rs = pl.ds(pl.multiple_of(i * _BQS, _BQS), _BQS)
                qn = _unit(q_ref[hh, :, rs].astype(jnp.float32)).astype(jnp.bfloat16)
                s = jnp.dot(kn_ref[...], qn, preferred_element_type=jnp.float32) * tval
                p = jnp.exp2(s - jnp.max(s, axis=0, keepdims=True))
                l = jnp.sum(p, axis=0, keepdims=True)
                acc = jnp.dot(v_ref[hh], p.astype(jnp.bfloat16), preferred_element_type=jnp.float32)
                o_ref[hh, :, rs] = (acc / l).astype(o_ref.dtype)
                return c

            jax.lax.fori_loop(0, S // _BQS, rtile, 0)
            return carry

        jax.lax.fori_loop(0, _HPS, head, 0)


@jax.jit
def pallas_standalone__qk_norm__prompt_kernel(
    q: jax.Array,
    k: jax.Array,
    v: jax.Array,
    t: jax.Array,
):
    B, H, S, Dh = q.shape
    BH = B * H
    assert Dh == 32 and S % _BQ == 0 and H % _HPS == 0 and _CK == _DT and _BQ <= 1024
    qt = jnp.swapaxes(q, 2, 3).reshape(BH, Dh, S)
    kt = jnp.swapaxes(k, 2, 3).reshape(BH, Dh, S)
    vt = jnp.swapaxes(v, 2, 3).reshape(BH, Dh, S)
    spec = pl.BlockSpec((_HPS, Dh, S), lambda g: (g, 0, 0))
    nxt = lambda g: (jnp.minimum((g + 1) * _HPS, BH - 1), 0, 0)
    out = pl.pallas_call(
        _kernel,
        grid=(BH // _HPS,),
        in_specs=[pl.BlockSpec(memory_space=pltpu.SMEM), spec, spec, spec,
                  pl.BlockSpec((1, Dh, _BQ), nxt), pl.BlockSpec((1, Dh, S), nxt)],
        out_specs=spec,
        out_shape=jax.ShapeDtypeStruct((BH, Dh, S), q.dtype),
        scratch_shapes=[
            pltpu.VMEM((S, 4 * Dh), jnp.int8),
            pltpu.VMEM((S, Dh), jnp.bfloat16),
            pltpu.VMEM((4 * Dh, _BQ), jnp.int8),
            pltpu.VMEM((1, _BQ), jnp.float32),
            pltpu.SMEM((1,), jnp.int32),
        ],
        compiler_params=pltpu.CompilerParams(
            dimension_semantics=("arbitrary",),
            vmem_limit_bytes=100 * 1024 * 1024,
        ),
    )(t.astype(jnp.float32), qt, kt, vt, qt, kt)
    return jnp.swapaxes(out.reshape(B, H, Dh, S), 2, 3)
```

```python
import jax
import jax.numpy as jnp
import jax.experimental.pallas as pl
import jax.experimental.pallas.tpu as pltpu

_LOG2E = 1.4426950408889634
_EPS = 1e-6
_T_SAFE = 16.0
_MAGIC = 12582912.0

_HPS = 4
_BQ = 1024
_CK = 128
_DT = 128
_BQS = 512

_SCHED = dict(qs=[0], ks=[2], qd=[4, 5, 6, 7, 8, 9, 10, 11],
              kd=[6, 7, 8, 9, 10, 11, 12, 13])


def _unit(x):
    return x / (jnp.sqrt(jnp.sum(x * x, axis=0, keepdims=True)) + _EPS)


def _compact(x):
    rows = jax.lax.broadcasted_iota(jnp.int32, (8, 128), 0)
    c = jnp.broadcast_to(x[:, 0:128], (8, 128))
    for s in range(1, x.shape[1] // 128):
        c = jnp.where(rows == s, jnp.broadcast_to(x[:, s * 128:(s + 1) * 128], (8, 128)), c)
    return c


def _expand(c, n):
    return jnp.concatenate([c[s:s + 1, :] for s in range(n)], axis=1)


def _inv_norm(ss):
    y = jax.lax.rsqrt(jnp.maximum(ss, 1e-36))
    return y * pltpu.reciprocal(1.0 + _EPS * y, approx=True)


def _k_scale(kf):
    ss = _compact(jnp.sum(kf * kf, axis=0, keepdims=True))
    return _expand(_inv_norm(ss) * 4064.0, kf.shape[1] // 128)


def _k_digits(kf, inv):
    t = pltpu.bitcast(kf * inv + (_MAGIC + 8.0), jnp.int32)
    planes = [t >> 5, (t + 16) >> 5, (t & 15) - 8, (t + 120) >> 8]
    return jnp.concatenate(planes, axis=0).T.astype(jnp.int8)


def _q_scale(qf):
    n = qf.shape[1] // 128
    sq = qf * qf
    inv = _inv_norm(_compact(jnp.sum(sq, axis=0, keepdims=True)))
    m2 = jnp.clip(_compact(jnp.max(sq, axis=0, keepdims=True)), 1e-36, 3.4028234e38)
    y = jax.lax.rsqrt(m2)
    return _expand(y * 2032.0, n), _expand(m2 * y * inv, n)


def _q_digits(qf, r):
    t = pltpu.bitcast(qf * r + (_MAGIC + 4.0), jnp.int32)
    planes = [t >> 4, (t + 8) >> 4, (t + 124) >> 8, (t & 7) - 4]
    return jnp.concatenate(planes, axis=0).astype(jnp.int8)


def _zero_from(*vals):
    acc = None
    for v in vals:
        w = pltpu.bitcast(v, jnp.int32)
        if w.shape[0] == 1:
            w = jnp.broadcast_to(w, (8, w.shape[1]))
        for i in range(0, w.shape[0], 8):
            for j in range(0, w.shape[1], 128):
                x = w[i:i + 8, j:j + 128]
                acc = x if acc is None else acc | x
    zero = jnp.minimum(jax.lax.shift_right_logical(acc, 1), 0)
    return pltpu.bitcast(zero, jnp.float32)


def _kernel(t_ref, q_ref, k_ref, v_ref, qx_ref, kx_ref, o_ref,
            kd_ref, kn_ref, qd_ref, qm_ref, flag_ref):
    S = k_ref.shape[-1]
    H = t_ref.shape[0]
    step = pl.program_id(0)
    h0 = (step * _HPS) % H

    @pl.when(step == 0)
    def _prologue():
        tmax = jnp.abs(t_ref[0].astype(jnp.float32))
        for h in range(1, H):
            tmax = jnp.maximum(tmax, jnp.abs(t_ref[h].astype(jnp.float32)))
        flag_ref[0] = (tmax <= _T_SAFE).astype(jnp.int32)
        for i in range(S // _BQ):
            kf = k_ref[0, :, pl.ds(i * _BQ, _BQ)].astype(jnp.float32)
            kd_ref[pl.ds(i * _BQ, _BQ), :] = _k_digits(kf, _k_scale(kf))
        qf = q_ref[0, :, pl.ds(0, _BQ)].astype(jnp.float32)
        r, m = _q_scale(qf)
        qd_ref[...] = _q_digits(qf, r)
        qm_ref[...] = m

    safe = flag_ref[0] == 1

    @pl.when(safe)
    def _bounded_logits():
        n_c, n_r, n_d = S // _CK, S // _BQ, _BQ // _DT
        items = [(hh, i, c) for hh in range(_HPS) for i in range(n_r) for c in range(n_c)]
        P, L, ACC, SC, QD, QS, KS, KD = {}, {}, {}, {}, {}, {}, {}, {}
        at = {}
        for kind, pos in _SCHED.items():
            for j, c in enumerate(pos):
                at.setdefault(c, []).append((kind, j))

        def k_src(hh):
            return k_ref.at[hh + 1] if hh + 1 < _HPS else kx_ref.at[0]

        def q_src(hh, i):
            if i + 1 < n_r:
                return q_ref.at[hh], (i + 1) * _BQ
            return (q_ref.at[hh + 1] if hh + 1 < _HPS else qx_ref.at[0]), 0

        def prepare(n):
            hh, i, c = items[n]
            u = hh * n_r + i
            q_nxt, base = q_src(hh, i)
            outs = []
            for kind, j in at.get(c, []):
                cols = slice(j * _DT, (j + 1) * _DT)
                if kind == "ks":
                    KS[u] = _k_scale(k_src(hh)[:, pl.ds(i * _BQ, _BQ)].astype(jnp.float32))
                    outs.append(KS[u])
                elif kind == "qs":
                    QS[u] = _q_scale(q_nxt[:, pl.ds(base, _BQ)].astype(jnp.float32))
                    outs += list(QS[u])
                elif kind == "kd":
                    kf = k_src(hh)[:, pl.ds(i * _BQ + j * _DT, _DT)].astype(jnp.float32)
                    KD[hh + 1, i * n_d + j] = _k_digits(kf, KS[u][:, cols])
                    outs.append(KD[hh + 1, i * n_d + j])
                else:
                    qf = q_nxt[:, pl.ds(base + j * _DT, _DT)].astype(jnp.float32)
                    QD[u + 1, j] = _q_digits(qf, QS[u][0][:, cols])
                    outs.append(QD[u + 1, j])
            return outs

        def scores(n):
            hh, i, c = items[n]
            u = hh * n_r + i
            if c == 0:
                if u == 0:
                    QD[u], m = qd_ref[...], qm_ref[...]
                else:
                    QD[u] = jnp.concatenate([QD[u, j] for j in range(n_d)], axis=1)
                    m = QS[u - 1][1]
                SC[u] = m * (t_ref[h0 + hh].astype(jnp.float32) * (_LOG2E / 32258.0))
            kd = kd_ref[pl.ds(c * _CK, _CK), :] if hh == 0 else KD[hh, c]
            s = jnp.dot(kd, QD[u], preferred_element_type=jnp.int32)
            p = jnp.exp2(s.astype(jnp.float32) * SC[u])
            P[n] = p.astype(jnp.bfloat16)
            ls = jnp.sum(p.reshape(_CK // 8, 8, _BQ), axis=0)
            L[hh, i] = ls if c == 0 else L[hh, i] + ls

        def values(n):
            hh, i, c = items[n]
            a = jnp.dot(v_ref[hh, :, pl.ds(c * _CK, _CK)], P.pop(n),
                        preferred_element_type=jnp.float32)
            outs = prepare(n)
            if outs:
                top = jnp.concatenate([a[:8, :-128], a[:8, -128:] + _zero_from(*outs)], axis=1)
                a = jnp.concatenate([top, a[8:]], axis=0)
            ACC[hh, i] = a if c == 0 else ACC[hh, i] + a
            if c == n_c - 1:
                l = jnp.sum(L.pop((hh, i)), axis=0, keepdims=True)
                o_ref[hh, :, pl.ds(i * _BQ, _BQ)] = (ACC.pop((hh, i)) / l).astype(o_ref.dtype)

        for n in range(len(items) + 1):
            if n < len(items):
                scores(n)
            if n >= 1:
                values(n - 1)

        for j in range(S // _DT):
            kd_ref[pl.ds(j * _DT, _DT), :] = KD[_HPS, j]
        for j in range(n_d):
            qd_ref[:, pl.ds(j * _DT, _DT)] = QD[_HPS * n_r, j]
        qm_ref[...] = QS[_HPS * n_r - 1][1]

    @pl.when(jnp.logical_not(safe))
    def _true_max():
        def head(hh, carry):
            kn_ref[...] = _unit(k_ref[hh].astype(jnp.float32)).T.astype(jnp.bfloat16)
            tval = t_ref[h0 + hh].astype(jnp.float32) * _LOG2E

            def rtile(i, c):
                rs = pl.ds(pl.multiple_of(i * _BQS, _BQS), _BQS)
                qn = _unit(q_ref[hh, :, rs].astype(jnp.float32)).astype(jnp.bfloat16)
                s = jnp.dot(kn_ref[...], qn, preferred_element_type=jnp.float32) * tval
                p = jnp.exp2(s - jnp.max(s, axis=0, keepdims=True))
                l = jnp.sum(p, axis=0, keepdims=True)
                acc = jnp.dot(v_ref[hh], p.astype(jnp.bfloat16), preferred_element_type=jnp.float32)
                o_ref[hh, :, rs] = (acc / l).astype(o_ref.dtype)
                return c

            jax.lax.fori_loop(0, S // _BQS, rtile, 0)
            return carry

        jax.lax.fori_loop(0, _HPS, head, 0)


@jax.jit
def pallas_standalone__qk_norm__prompt_kernel(
    q: jax.Array,
    k: jax.Array,
    v: jax.Array,
    t: jax.Array,
):
    B, H, S, Dh = q.shape
    BH = B * H
    assert Dh == 32 and S % _BQ == 0 and H % _HPS == 0 and _CK == _DT and _BQ <= 1024
    qt = jnp.swapaxes(q, 2, 3).reshape(BH, Dh, S)
    kt = jnp.swapaxes(k, 2, 3).reshape(BH, Dh, S)
    vt = jnp.swapaxes(v, 2, 3).reshape(BH, Dh, S)
    spec = pl.BlockSpec((_HPS, Dh, S), lambda g: (g, 0, 0))
    nxt = lambda g: (jnp.minimum((g + 1) * _HPS, BH - 1), 0, 0)
    out = pl.pallas_call(
        _kernel,
        grid=(BH // _HPS,),
        in_specs=[pl.BlockSpec(memory_space=pltpu.SMEM), spec, spec, spec,
                  pl.BlockSpec((1, Dh, _BQ), nxt), pl.BlockSpec((1, Dh, S), nxt)],
        out_specs=spec,
        out_shape=jax.ShapeDtypeStruct((BH, Dh, S), q.dtype),
        scratch_shapes=[
            pltpu.VMEM((S, 4 * Dh), jnp.int8),
            pltpu.VMEM((S, Dh), jnp.bfloat16),
            pltpu.VMEM((4 * Dh, _BQ), jnp.int8),
            pltpu.VMEM((1, _BQ), jnp.float32),
            pltpu.SMEM((1,), jnp.int32),
        ],
        compiler_params=pltpu.CompilerParams(
            dimension_semantics=("arbitrary",),
            vmem_limit_bytes=100 * 1024 * 1024,
        ),
    )(t, qt, kt, vt, qt, kt)
    return jnp.swapaxes(out.reshape(B, H, Dh, S), 2, 3)
```

```python
import jax
import jax.numpy as jnp
import jax.experimental.pallas as pl
import jax.experimental.pallas.tpu as pltpu

_LOG2E = 1.4426950408889634
_EPS = 1e-6
_T_SAFE = 16.0
_MAGIC = 12582912.0

_HPS = 4
_BQ = 1024
_CK = 128
_DT = 128
_BQS = 512

_SCHED = dict(qs=[0], ks=[2], qd=[4, 5, 6, 7, 8, 9, 10, 11],
              kd=[6, 7, 8, 9, 10, 11, 12, 13])


def _unit(x):
    return x / (jnp.sqrt(jnp.sum(x * x, axis=0, keepdims=True)) + _EPS)


def _compact(x):
    rows = jax.lax.broadcasted_iota(jnp.int32, (8, 128), 0)
    c = jnp.broadcast_to(x[:, 0:128], (8, 128))
    for s in range(1, x.shape[1] // 128):
        c = jnp.where(rows == s, jnp.broadcast_to(x[:, s * 128:(s + 1) * 128], (8, 128)), c)
    return c


def _expand(c, n):
    return jnp.concatenate([c[s:s + 1, :] for s in range(n)], axis=1)


def _inv_norm(ss):
    y = jax.lax.rsqrt(jnp.maximum(ss, 1e-36))
    return y * pltpu.reciprocal(1.0 + _EPS * y, approx=True)


def _k_scale(kf):
    ss = _compact(jnp.sum(kf * kf, axis=0, keepdims=True))
    return _expand(_inv_norm(ss) * 4064.0, kf.shape[1] // 128)


def _k_digits(kf, inv):
    t = pltpu.bitcast(kf * inv + (_MAGIC + 8.0), jnp.int32)
    planes = [t >> 5,
              (t + 16) >> 5,
              (t & 15) - 8,
              (t + 120) >> 8]
    return jnp.concatenate(planes, axis=0).T.astype(jnp.int8)


def _q_scale(qf):
    n = qf.shape[1] // 128
    sq = qf * qf
    inv = _inv_norm(_compact(jnp.sum(sq, axis=0, keepdims=True)))
    m2 = jnp.clip(_compact(jnp.max(sq, axis=0, keepdims=True)), 1e-36, 3.4028234e38)
    y = jax.lax.rsqrt(m2)
    return _expand(y * 2032.0, n), _expand(m2 * y * inv, n)


def _q_digits(qf, r):
    t = pltpu.bitcast(qf * r + (_MAGIC + 4.0), jnp.int32)
    planes = [t >> 4,
              (t + 8) >> 4,
              (t + 124) >> 8,
              (t & 7) - 4]
    return jnp.concatenate(planes, axis=0).astype(jnp.int8)


def _zero_from(*vals):
    acc = None
    for v in vals:
        w = pltpu.bitcast(v, jnp.int32)
        if w.shape[0] == 1:
            w = jnp.broadcast_to(w, (8, w.shape[1]))
        for i in range(0, w.shape[0], 8):
            for j in range(0, w.shape[1], 128):
                x = w[i:i + 8, j:j + 128]
                acc = x if acc is None else acc | x
    zero = jnp.minimum(jax.lax.shift_right_logical(acc, 1), 0)
    return pltpu.bitcast(zero, jnp.float32)


def _kernel(t_ref, q_ref, k_ref, v_ref, qx_ref, kx_ref, o_ref,
            kd_ref, kn_ref, qd_ref, qm_ref, flag_ref):
    S = k_ref.shape[-1]
    H = t_ref.shape[0]
    step = pl.program_id(0)
    h0 = (step * _HPS) % H

    @pl.when(step == 0)
    def _prologue():
        tmax = jnp.abs(t_ref[0].astype(jnp.float32))
        for h in range(1, H):
            tmax = jnp.maximum(tmax, jnp.abs(t_ref[h].astype(jnp.float32)))
        flag_ref[0] = (tmax <= _T_SAFE).astype(jnp.int32)
        for i in range(S // _BQ):
            kf = k_ref[0, :, pl.ds(i * _BQ, _BQ)].astype(jnp.float32)
            kd_ref[pl.ds(i * _BQ, _BQ), :] = _k_digits(kf, _k_scale(kf))
        qf = q_ref[0, :, pl.ds(0, _BQ)].astype(jnp.float32)
        r, m = _q_scale(qf)
        qd_ref[...] = _q_digits(qf, r)
        qm_ref[...] = m

    safe = flag_ref[0] == 1

    @pl.when(safe)
    def _bounded_logits():
        n_c, n_r, n_d = S // _CK, S // _BQ, _BQ // _DT
        items = [(hh, i, c) for hh in range(_HPS) for i in range(n_r) for c in range(n_c)]
        P, L, ACC, SC, QD, QS, KS, KD = {}, {}, {}, {}, {}, {}, {}, {}
        at = {}
        for kind, pos in _SCHED.items():
            for j, c in enumerate(pos):
                at.setdefault(c, []).append((kind, j))

        def k_src(hh):
            return k_ref.at[hh + 1] if hh + 1 < _HPS else kx_ref.at[0]

        def q_src(hh, i):
            if i + 1 < n_r:
                return q_ref.at[hh], (i + 1) * _BQ
            return (q_ref.at[hh + 1] if hh + 1 < _HPS else qx_ref.at[0]), 0

        def prepare(n):
            hh, i, c = items[n]
            u = hh * n_r + i
            q_nxt, base = q_src(hh, i)
            outs = []
            for kind, j in at.get(c, []):
                cols = slice(j * _DT, (j + 1) * _DT)
                if kind == "ks":
                    KS[u] = _k_scale(k_src(hh)[:, pl.ds(i * _BQ, _BQ)].astype(jnp.float32))
                    outs.append(KS[u])
                elif kind == "qs":
                    QS[u] = _q_scale(q_nxt[:, pl.ds(base, _BQ)].astype(jnp.float32))
                    outs += list(QS[u])
                elif kind == "kd":
                    kf = k_src(hh)[:, pl.ds(i * _BQ + j * _DT, _DT)].astype(jnp.float32)
                    KD[hh + 1, i * n_d + j] = _k_digits(kf, KS[u][:, cols])
                    outs.append(KD[hh + 1, i * n_d + j])
                else:
                    qf = q_nxt[:, pl.ds(base + j * _DT, _DT)].astype(jnp.float32)
                    QD[u + 1, j] = _q_digits(qf, QS[u][0][:, cols])
                    outs.append(QD[u + 1, j])
            return outs

        def scores(n):
            hh, i, c = items[n]
            u = hh * n_r + i
            if c == 0:
                if u == 0:
                    QD[u], m = qd_ref[...], qm_ref[...]
                else:
                    QD[u] = jnp.concatenate([QD[u, j] for j in range(n_d)], axis=1)
                    m = QS[u - 1][1]
                SC[u] = m * (t_ref[h0 + hh].astype(jnp.float32) * (_LOG2E / 32258.0))
            kd = kd_ref[pl.ds(c * _CK, _CK), :] if hh == 0 else KD[hh, c]
            s = jnp.dot(kd, QD[u], preferred_element_type=jnp.int32)
            p = jnp.exp2(s.astype(jnp.float32) * SC[u])
            P[n] = p.astype(jnp.bfloat16)
            ls = jnp.sum(p.reshape(_CK // 8, 8, _BQ), axis=0)
            L[hh, i] = ls if c == 0 else L[hh, i] + ls

        def values(n):
            hh, i, c = items[n]
            a = jnp.dot(v_ref[hh, :, pl.ds(c * _CK, _CK)], P.pop(n),
                        preferred_element_type=jnp.float32)
            outs = prepare(n)
            if outs:
                top = jnp.concatenate([a[:8, :-128], a[:8, -128:] + _zero_from(*outs)], axis=1)
                a = jnp.concatenate([top, a[8:]], axis=0)
            ACC[hh, i] = a if c == 0 else ACC[hh, i] + a
            if c == n_c - 1:
                l = jnp.sum(L.pop((hh, i)), axis=0, keepdims=True)
                o_ref[hh, :, pl.ds(i * _BQ, _BQ)] = (ACC.pop((hh, i)) / l).astype(o_ref.dtype)

        for n in range(len(items) + 1):
            if n < len(items):
                scores(n)
            if n >= 1:
                values(n - 1)

        for j in range(S // _DT):
            kd_ref[pl.ds(j * _DT, _DT), :] = KD[_HPS, j]
        for j in range(n_d):
            qd_ref[:, pl.ds(j * _DT, _DT)] = QD[_HPS * n_r, j]
        qm_ref[...] = QS[_HPS * n_r - 1][1]

    @pl.when(jnp.logical_not(safe))
    def _true_max():
        def head(hh, carry):
            kn_ref[...] = _unit(k_ref[hh].astype(jnp.float32)).T.astype(jnp.bfloat16)
            tval = t_ref[h0 + hh].astype(jnp.float32) * _LOG2E

            def rtile(i, c):
                rs = pl.ds(pl.multiple_of(i * _BQS, _BQS), _BQS)
                qn = _unit(q_ref[hh, :, rs].astype(jnp.float32)).astype(jnp.bfloat16)
                s = jnp.dot(kn_ref[...], qn, preferred_element_type=jnp.float32) * tval
                p = jnp.exp2(s - jnp.max(s, axis=0, keepdims=True))
                l = jnp.sum(p, axis=0, keepdims=True)
                acc = jnp.dot(v_ref[hh], p.astype(jnp.bfloat16), preferred_element_type=jnp.float32)
                o_ref[hh, :, rs] = (acc / l).astype(o_ref.dtype)
                return c

            jax.lax.fori_loop(0, S // _BQS, rtile, 0)
            return carry

        jax.lax.fori_loop(0, _HPS, head, 0)


@jax.jit
def pallas_standalone__qk_norm__prompt_kernel(
    q: jax.Array,
    k: jax.Array,
    v: jax.Array,
    t: jax.Array,
):
    B, H, S, Dh = q.shape
    BH = B * H
    assert Dh == 32 and S % _BQ == 0 and H % _HPS == 0 and _CK == _DT and _BQ <= 1024
    qt = jnp.swapaxes(q, 2, 3).reshape(BH, Dh, S)
    kt = jnp.swapaxes(k, 2, 3).reshape(BH, Dh, S)
    vt = jnp.swapaxes(v, 2, 3).reshape(BH, Dh, S)
    spec = pl.BlockSpec((_HPS, Dh, S), lambda g: (g, 0, 0))
    nxt = lambda g: (jnp.minimum((g + 1) * _HPS, BH - 1), 0, 0)
    out = pl.pallas_call(
        _kernel,
        grid=(BH // _HPS,),
        in_specs=[pl.BlockSpec(memory_space=pltpu.SMEM), spec, spec, spec,
                  pl.BlockSpec((1, Dh, _BQ), nxt), pl.BlockSpec((1, Dh, S), nxt)],
        out_specs=spec,
        out_shape=jax.ShapeDtypeStruct((BH, Dh, S), q.dtype),
        scratch_shapes=[
            pltpu.VMEM((S, 4 * Dh), jnp.int8),
            pltpu.VMEM((S, Dh), jnp.bfloat16),
            pltpu.VMEM((4 * Dh, _BQ), jnp.int8),
            pltpu.VMEM((1, _BQ), jnp.float32),
            pltpu.SMEM((1,), jnp.int32),
        ],
        compiler_params=pltpu.CompilerParams(
            dimension_semantics=("arbitrary",),
            vmem_limit_bytes=100 * 1024 * 1024,
        ),
    )(t, qt, kt, vt, qt, kt)
    return jnp.swapaxes(out.reshape(B, H, Dh, S), 2, 3)
```

```python
import jax
import jax.numpy as jnp
import jax.experimental.pallas as pl
import jax.experimental.pallas.tpu as pltpu

_LOG2E = 1.4426950408889634
_EPS = 1e-6
_T_SAFE = 16.0
_MAGIC = 12582912.0

_HPS = 8
_BQ = 1024
_CK = 128
_DT = 128
_BQS = 512

_SCHED = dict(q_sums=[0], q_scale=[2], k_sums=[3], k_scale=[5],
              q_digits=[5, 6, 7, 8, 9, 10, 11, 12],
              k_digits=[7, 8, 9, 10, 11, 12, 14, 15])


def _unit(x):
    return x / (jnp.sqrt(jnp.sum(x * x, axis=0, keepdims=True)) + _EPS)


def _compact(x):
    rows = jax.lax.broadcasted_iota(jnp.int32, (8, 128), 0)
    c = jnp.broadcast_to(x[:, 0:128], (8, 128))
    for s in range(1, x.shape[1] // 128):
        c = jnp.where(rows == s, jnp.broadcast_to(x[:, s * 128:(s + 1) * 128], (8, 128)), c)
    return c


def _expand(c, n):
    return jnp.concatenate([c[s:s + 1, :] for s in range(n)], axis=1)


def _inv_norm(ss):
    y = jax.lax.rsqrt(jnp.maximum(ss, 1e-36))
    return y * pltpu.reciprocal(1.0 + _EPS * y, approx=True)


def _k_sums(kf):
    return _compact(jnp.sum(kf * kf, axis=0, keepdims=True))


def _k_scale(ss, n):
    return _expand(_inv_norm(ss) * 4064.0, n)


def _k_digits(kf, inv):
    t = pltpu.bitcast(kf * inv + (_MAGIC + 8.0), jnp.int32)
    planes = [t >> 5,
              (t + 16) >> 5,
              (t & 15) - 8,
              (t + 120) >> 8]
    return jnp.concatenate(planes, axis=0).astype(jnp.int16).T.astype(jnp.int8)


def _q_sums(qf):
    sq = qf * qf
    return (_compact(jnp.sum(sq, axis=0, keepdims=True)),
            _compact(jnp.max(sq, axis=0, keepdims=True)))


def _q_scale(ss, m2, n):
    m2 = jnp.clip(m2, 1e-36, 3.4028234e38)
    y = jax.lax.rsqrt(m2)
    return _expand(y * 2032.0, n), _expand(m2 * y * _inv_norm(ss), n)


def _q_digits(qf, r):
    t = pltpu.bitcast(qf * r + (_MAGIC + 4.0), jnp.int32)
    planes = [t >> 4,
              (t + 8) >> 4,
              (t + 124) >> 8,
              (t & 7) - 4]
    return jnp.concatenate(planes, axis=0).astype(jnp.int8)


def _zero_from(*vals):
    acc = None
    for v in vals:
        w = pltpu.bitcast(v, jnp.int32)
        if w.shape[0] == 1:
            w = jnp.broadcast_to(w, (8, w.shape[1]))
        for i in range(0, w.shape[0], 8):
            for j in range(0, w.shape[1], 128):
                x = w[i:i + 8, j:j + 128]
                acc = x if acc is None else acc | x
    zero = jnp.minimum(jax.lax.shift_right_logical(acc, 1), 0)
    return pltpu.bitcast(zero, jnp.float32)


def _kernel(t_ref, q_ref, k_ref, v_ref, qx_ref, kx_ref, o_ref,
            kd_ref, kn_ref, qd_ref, qm_ref, flag_ref):
    S = k_ref.shape[-1]
    H = t_ref.shape[0]
    step = pl.program_id(0)
    h0 = (step * _HPS) % H
    n_t = _BQ // 128

    @pl.when(step == 0)
    def _prologue():
        tmax = jnp.abs(t_ref[0].astype(jnp.float32))
        for h in range(1, H):
            tmax = jnp.maximum(tmax, jnp.abs(t_ref[h].astype(jnp.float32)))
        flag_ref[0] = (tmax <= _T_SAFE).astype(jnp.int32)
        for i in range(S // _BQ):
            kf = k_ref[0, :, pl.ds(i * _BQ, _BQ)].astype(jnp.float32)
            kd_ref[pl.ds(i * _BQ, _BQ), :] = _k_digits(kf, _k_scale(_k_sums(kf), n_t))
        qf = q_ref[0, :, pl.ds(0, _BQ)].astype(jnp.float32)
        r, m = _q_scale(*_q_sums(qf), n_t)
        qd_ref[...] = _q_digits(qf, r)
        qm_ref[...] = m

    safe = flag_ref[0] == 1

    @pl.when(safe)
    def _bounded_logits():
        n_c, n_r, n_d = S // _CK, S // _BQ, _BQ // _DT
        items = [(hh, i, c) for hh in range(_HPS) for i in range(n_r) for c in range(n_c)]
        P, L, ACC, SC, QD, QS, KS, KD, T = {}, {}, {}, {}, {}, {}, {}, {}, {}
        last = []
        at = {}
        for kind, pos in _SCHED.items():
            for j, c in enumerate(pos):
                at.setdefault(c, []).append((kind, j))

        def k_src(hh):
            return k_ref.at[hh + 1] if hh + 1 < _HPS else kx_ref.at[0]

        def q_src(hh, i):
            if i + 1 < n_r:
                return q_ref.at[hh], (i + 1) * _BQ
            return (q_ref.at[hh + 1] if hh + 1 < _HPS else qx_ref.at[0]), 0

        def prepare(n):
            hh, i, c = items[n]
            u = hh * n_r + i
            q_nxt, base = q_src(hh, i)
            outs = []
            for kind, j in at.get(c, []):
                cols = slice(j * _DT, (j + 1) * _DT)
                if kind == "k_sums":
                    T[kind, u] = _k_sums(k_src(hh)[:, pl.ds(i * _BQ, _BQ)].astype(jnp.float32))
                    outs.append(T[kind, u])
                elif kind == "q_sums":
                    T[kind, u] = _q_sums(q_nxt[:, pl.ds(base, _BQ)].astype(jnp.float32))
                    outs += list(T[kind, u])
                elif kind == "k_scale":
                    KS[u] = _k_scale(T.pop(("k_sums", u)), n_t)
                    outs.append(KS[u])
                elif kind == "q_scale":
                    QS[u] = _q_scale(*T.pop(("q_sums", u)), n_t)
                    outs += list(QS[u])
                elif kind == "k_digits":
                    kf = k_src(hh)[:, pl.ds(i * _BQ + j * _DT, _DT)].astype(jnp.float32)
                    KD[hh + 1, i * n_d + j] = _k_digits(kf, KS[u][:, cols])
                    outs.append(KD[hh + 1, i * n_d + j])
                else:
                    qf = q_nxt[:, pl.ds(base + j * _DT, _DT)].astype(jnp.float32)
                    QD[u + 1, j] = _q_digits(qf, QS[u][0][:, cols])
                    outs.append(QD[u + 1, j])
            return outs

        def scores(n):
            hh, i, c = items[n]
            u = hh * n_r + i
            if c == 0:
                if u == 0:
                    QD[u], m = qd_ref[...], qm_ref[...]
                else:
                    QD[u] = jnp.concatenate([QD[u, j] for j in range(n_d)], axis=1)
                    m = QS[u - 1][1]
                SC[u] = m * (t_ref[h0 + hh].astype(jnp.float32) * (_LOG2E / 32258.0))
            kd = kd_ref[pl.ds(c * _CK, _CK), :] if hh == 0 else KD[hh, c]
            s = jnp.dot(kd, QD[u], preferred_element_type=jnp.int32)
            p = jnp.exp2(s.astype(jnp.float32) * SC[u])
            P[n] = p.astype(jnp.bfloat16)
            ls = jnp.sum(p.reshape(_CK // 8, 8, _BQ), axis=0)
            L[hh, i] = ls if c == 0 else L[hh, i] + ls

        def values(n):
            hh, i, c = items[n]
            a = jnp.dot(v_ref[hh, :, pl.ds(c * _CK, _CK)], P.pop(n),
                        preferred_element_type=jnp.float32)
            outs = prepare(n)
            if outs:
                top = jnp.concatenate([a[:8, :-128], a[:8, -128:] + _zero_from(*outs)], axis=1)
                a = jnp.concatenate([top, a[8:]], axis=0)
            if c == 0 and last:
                top = jnp.concatenate([a[:8, :128] + _zero_from(last.pop()), a[:8, 128:]], axis=1)
                a = jnp.concatenate([top, a[8:]], axis=0)
            ACC[hh, i] = a if c == 0 else ACC[hh, i] + a
            if c == n_c - 1:
                acc = ACC.pop((hh, i))
                last.append(acc[:8, -128:])
                l = jnp.sum(L.pop((hh, i)), axis=0, keepdims=True)
                out = acc * pltpu.reciprocal(l, approx=True)
                o_ref[hh, :, pl.ds(i * _BQ, _BQ)] = out.astype(o_ref.dtype)

        for n in range(len(items) + 1):
            if n < len(items):
                scores(n)
            if n >= 1:
                values(n - 1)

        for j in range(S // _DT):
            kd_ref[pl.ds(j * _DT, _DT), :] = KD[_HPS, j]
        for j in range(n_d):
            qd_ref[:, pl.ds(j * _DT, _DT)] = QD[_HPS * n_r, j]
        qm_ref[...] = QS[_HPS * n_r - 1][1]

    @pl.when(jnp.logical_not(safe))
    def _true_max():
        def head(hh, carry):
            kn_ref[...] = _unit(k_ref[hh].astype(jnp.float32)).T.astype(jnp.bfloat16)
            tval = t_ref[h0 + hh].astype(jnp.float32) * _LOG2E

            def rtile(i, c):
                rs = pl.ds(pl.multiple_of(i * _BQS, _BQS), _BQS)
                qn = _unit(q_ref[hh, :, rs].astype(jnp.float32)).astype(jnp.bfloat16)
                s = jnp.dot(kn_ref[...], qn, preferred_element_type=jnp.float32) * tval
                p = jnp.exp2(s - jnp.max(s, axis=0, keepdims=True))
                l = jnp.sum(p, axis=0, keepdims=True)
                acc = jnp.dot(v_ref[hh], p.astype(jnp.bfloat16), preferred_element_type=jnp.float32)
                o_ref[hh, :, rs] = (acc / l).astype(o_ref.dtype)
                return c

            jax.lax.fori_loop(0, S // _BQS, rtile, 0)
            return carry

        jax.lax.fori_loop(0, _HPS, head, 0)


@jax.jit
def pallas_standalone__qk_norm__prompt_kernel(
    q: jax.Array,
    k: jax.Array,
    v: jax.Array,
    t: jax.Array,
):
    B, H, S, Dh = q.shape
    BH = B * H
    assert Dh == 32 and S % _BQ == 0 and H % _HPS == 0 and _CK == _DT and _BQ <= 1024
    qt = jnp.swapaxes(q, 2, 3).reshape(BH, Dh, S)
    kt = jnp.swapaxes(k, 2, 3).reshape(BH, Dh, S)
    vt = jnp.swapaxes(v, 2, 3).reshape(BH, Dh, S)
    spec = pl.BlockSpec((_HPS, Dh, S), lambda g: (g, 0, 0))
    nxt = lambda g: (jnp.minimum((g + 1) * _HPS, BH - 1), 0, 0)
    out = pl.pallas_call(
        _kernel,
        grid=(BH // _HPS,),
        in_specs=[pl.BlockSpec(memory_space=pltpu.SMEM), spec, spec, spec,
                  pl.BlockSpec((1, Dh, _BQ), nxt), pl.BlockSpec((1, Dh, S), nxt)],
        out_specs=spec,
        out_shape=jax.ShapeDtypeStruct((BH, Dh, S), q.dtype),
        scratch_shapes=[
            pltpu.VMEM((S, 4 * Dh), jnp.int8),
            pltpu.VMEM((S, Dh), jnp.bfloat16),
            pltpu.VMEM((4 * Dh, _BQ), jnp.int8),
            pltpu.VMEM((1, _BQ), jnp.float32),
            pltpu.SMEM((1,), jnp.int32),
        ],
        compiler_params=pltpu.CompilerParams(
            dimension_semantics=("arbitrary",),
            vmem_limit_bytes=100 * 1024 * 1024,
        ),
    )(t, qt, kt, vt, qt, kt)
    return jnp.swapaxes(out.reshape(B, H, Dh, S), 2, 3)
```
